```python
import os as _os
_os.environ.setdefault("JAX_PLATFORMS", "cpu")
import jax
import jax.numpy as jnp

def _softmax(x, axis=-1):
    return jax.nn.softmax(x, axis=axis)
def _gelu(x):
    return jax.nn.gelu(x, approximate=True)
def _silu(x):
    return jax.nn.silu(x)
def _sigmoid(x):
    return jax.nn.sigmoid(x)
def _layernorm(x, axis=-1, eps=1e-5):
    m = jnp.mean(x, axis=axis, keepdims=True)
    v = jnp.var(x, axis=axis, keepdims=True)
    return (x - m) / jnp.sqrt(v + eps)
def _scatter_add(tgt, idx, src, axis=0):
    return tgt.at[idx].add(src)
def _segment_sum(src, seg, n):
    return jax.ops.segment_sum(src, seg, n)
class _Rng:
    def __init__(self, key):
        self._k = key
    def _next(self):
        self._k, sub = jax.random.split(self._k)
        return sub
    def normal(self, shape):
        return jax.random.normal(self._next(), shape, dtype=jnp.bfloat16)
    def randint(self, lo, hi, shape):
        return jax.random.randint(self._next(), shape, lo, hi, dtype=jnp.int32)
    def uniform(self, shape, lo=0.0, hi=1.0):
        return jax.random.uniform(self._next(), shape, jnp.bfloat16, lo, hi)
    def permutation(self, n):
        return jax.random.permutation(self._next(), n)


kernel_name = 'interleave_layers__spectral_gfnet__dense_activation_gelu__prompt'

def setup_inputs():
    _rng = _Rng(jax.random.key(int.from_bytes(__import__("os").urandom(4), "little")))
    _w = (lambda a: (lambda t: t.astype(jnp.bfloat16) if jnp.issubdtype(t.dtype, jnp.floating) else t)(jnp.asarray(a)))
    def _A_setup():
        B, S, D = 1, 2048, 640
        Df = D // 2 + 1
        return {
            "x": _w((lambda *s: _rng.normal(s) * 0.05)(B, S, D)),
            "w_r": _w((lambda *s: _rng.normal(s) * 0.2)(S, Df) * 0.02),
            "w_i": _w((lambda *s: _rng.normal(s) * 0.2)(S, Df) * 0.02),
        }
    _A_in = _A_setup()

    def _B_setup():
        B, S, D, F = 1, 2048, 640, 1728
        return {
            "x": _w((lambda *s: _rng.normal(s) * 0.05)(B, S, D)),
            "w1": _w((lambda *s: _rng.normal(s) * 0.1)(D, F) * (D ** -0.5)),
            "b1": _w((lambda *s: _rng.normal(s) * 0.1)(F) * 0.01),
            "w2": _w((lambda *s: _rng.normal(s) * 0.1)(F, D) * (F ** -0.5)),
            "b2": _w((lambda *s: _rng.normal(s) * 0.1)(D) * 0.01),
        }
    _B_in = _B_setup()

    return {
        "A_x": _A_in["x"],
        "A_w_r": _A_in["w_r"],
        "A_w_i": _A_in["w_i"],
        "B_x": _B_in["x"],
        "B_w1": _B_in["w1"],
        "B_b1": _B_in["b1"],
        "B_w2": _B_in["w2"],
        "B_b2": _B_in["b2"],
    }

def reference(A_x, A_w_r, A_w_i, B_x, B_w1, B_b1, B_w2, B_b2):
    def _A_ref(x, w_r, w_i):
        B, S, D = x.shape
        X = (lambda x, axes=(-2,-1): jnp.fft.rfft2(x.astype(jnp.float32), axes=axes))(x, axes=(-2, -1))
        W = w_r + 1j * w_i
        X = X * W
        y = (lambda x, s, axes=(-2,-1): jnp.fft.irfft2(x, s=s, axes=axes).astype(jnp.bfloat16))(X, (S, D), axes=(-2, -1))
        return y

    def _B_ref(x, w1, b1, w2, b2):
        h = jnp.einsum("bsd,df->bsf", x, w1) + b1
        h = _gelu(h)
        return jnp.einsum("bsf,fd->bsd", h, w2) + b2

    x = A_x
    x = x + _A_ref(_layernorm(x, axis=-1), A_w_r, A_w_i)
    x = x + _B_ref(_layernorm(x, axis=-1), B_w1, B_b1, B_w2, B_b2)
    x = x + _A_ref(_layernorm(x, axis=-1), A_w_r, A_w_i)
    x = x + _B_ref(_layernorm(x, axis=-1), B_w1, B_b1, B_w2, B_b2)
    return x
```

```python
import functools
import numpy as np
import jax
import jax.numpy as jnp
from jax import lax
import jax.experimental.pallas as pl
import jax.experimental.pallas.tpu as pltpu

S, D, F = 2048, 640, 1728
DF = D // 2 + 1
DP = 384
NB, BL = 16, 128
EPS = 1e-5
TM = 256


def _big(m):
    mr, mi = m.real, m.imag
    return np.block([[mr, mi], [-mi, mr]])


@functools.lru_cache(maxsize=None)
def _tables():
    d = np.arange(D)
    l = np.arange(DP)
    ang = 2.0 * np.pi * ((d[:, None] * l[None, :]) % D) / D
    fd = np.zeros((D, 2 * DP))
    fd[:, :DF] = np.cos(ang[:, :DF])
    fd[:, DP + 1:DP + DF - 1] = np.sin(ang[:, 1:DF - 1])
    gd = np.zeros((2 * DP, D))
    c = np.full(DF, 2.0)
    c[0] = c[DF - 1] = 1.0
    gd[:DF, :] = c[:, None] * np.cos(ang.T[:DF]) / (D * S)
    gd[DP + 1:DP + DF - 1, :] = 2.0 * np.sin(ang.T[1:DF - 1]) / (D * S)
    m1 = np.zeros((NB, 2 * BL, 2 * BL))
    m1i = np.zeros((NB, 2 * BL, 2 * BL))
    cc = np.arange(NB)
    for g in range(NB):
        m = np.zeros((BL, BL), np.complex128)
        for a in range(NB):
            for bl in range(8):
                n = BL * a + 8 * g + bl
                m[cc * 8 + bl, a * 8 + bl] = np.exp(-2j * np.pi * ((cc * n) % S) / S)
        m1[g] = _big(m)
        m1i[g] = _big(np.conj(m).T)
    b = np.arange(BL)
    f128 = np.exp(-2j * np.pi * ((b[:, None] * b[None, :]) % BL) / BL)
    bf = jnp.bfloat16
    return (np.asarray(fd, bf), np.asarray(gd, bf), np.asarray(m1, bf),
            np.asarray(m1i, bf), np.asarray(_big(f128), bf),
            np.asarray(_big(np.conj(f128)), bf))


def _ln(x):
    m = jnp.mean(x, axis=-1, keepdims=True)
    xc = x - m
    v = jnp.mean(xc * xc, axis=-1, keepdims=True)
    return xc * lax.rsqrt(v + EPS)


def _rb(x):
    return x.astype(jnp.bfloat16).astype(jnp.float32)


def _kernel(x_ref, wr_ref, wi_ref, w1_ref, b1_ref, w2_ref, b2_ref,
            fd_ref, gd_ref, m1_ref, m1i_ref, f_ref, fi_ref,
            o_ref, xs_ref, u_ref, wf_ref):
    xs_ref[...] = x_ref[...].astype(jnp.float32)
    for j in range(3):
        wf_ref[j] = wr_ref[:, j * 128:(j + 1) * 128].astype(jnp.float32)
        wf_ref[3 + j] = wi_ref[:, j * 128:(j + 1) * 128].astype(jnp.float32)

    def gfnet():
        def fwd(g, carry):
            off = pl.multiple_of(g * 8, 8)
            xg = jnp.concatenate(
                [xs_ref[pl.ds(a * BL + off, 8), :] for a in range(NB)], axis=0)
            xn = _ln(xg).astype(jnp.bfloat16)
            pq = jnp.dot(xn, fd_ref[...], preferred_element_type=jnp.float32)
            st = jnp.concatenate([pq[:, :DP], pq[:, DP:]], axis=0).astype(jnp.bfloat16)
            u = jnp.dot(m1_ref[g], st, preferred_element_type=jnp.float32)
            for c in range(NB):
                u_ref[0, pl.ds(c * BL + off, 8), :] = u[c * 8:(c + 1) * 8]
                u_ref[1, pl.ds(c * BL + off, 8), :] = u[BL + c * 8:BL + (c + 1) * 8]
            return carry
        lax.fori_loop(0, NB, fwd, 0)

        def mid(c, carry):
            r0 = pl.multiple_of(c * BL, BL)
            st = jnp.concatenate([u_ref[0, pl.ds(r0, BL), :],
                                  u_ref[1, pl.ds(r0, BL), :]], axis=0).astype(jnp.bfloat16)
            z = jnp.dot(f_ref[...], st, preferred_element_type=jnp.float32)
            p, q = z[:BL], z[BL:]
            wr = jnp.concatenate(
                [wf_ref[j, pl.ds(c, BL, stride=NB), :] for j in range(3)], axis=1)
            wi = jnp.concatenate(
                [wf_ref[3 + j, pl.ds(c, BL, stride=NB), :] for j in range(3)], axis=1)
            p2 = p * wr + q * wi
            q2 = q * wr - p * wi
            st2 = jnp.concatenate([p2, q2], axis=0).astype(jnp.bfloat16)
            v = jnp.dot(fi_ref[...], st2, preferred_element_type=jnp.float32)
            u_ref[0, pl.ds(r0, BL), :] = v[:BL]
            u_ref[1, pl.ds(r0, BL), :] = v[BL:]
            return carry
        lax.fori_loop(0, NB, mid, 0)

        def inv(g, carry):
            off = pl.multiple_of(g * 8, 8)
            st = jnp.concatenate(
                [u_ref[0, pl.ds(c * BL + off, 8), :] for c in range(NB)]
                + [u_ref[1, pl.ds(c * BL + off, 8), :] for c in range(NB)],
                axis=0).astype(jnp.bfloat16)
            t = jnp.dot(m1i_ref[g], st, preferred_element_type=jnp.float32)
            pq = jnp.concatenate([t[:BL], t[BL:]], axis=1).astype(jnp.bfloat16)
            y = _rb(jnp.dot(pq, gd_ref[...], preferred_element_type=jnp.float32))
            for a in range(NB):
                rows = pl.ds(a * BL + off, 8)
                xs_ref[rows, :] = _rb(xs_ref[rows, :] + y[a * 8:(a + 1) * 8])
            return carry
        lax.fori_loop(0, NB, inv, 0)

    def ffn():
        def body(i, carry):
            rows = pl.ds(pl.multiple_of(i * TM, TM), TM)
            x = xs_ref[rows, :]
            xn = _ln(x).astype(jnp.bfloat16)
            h = _rb(jnp.dot(xn, w1_ref[...], preferred_element_type=jnp.float32))
            h = _rb(h + b1_ref[...].astype(jnp.float32))
            h = jax.nn.gelu(h, approximate=True).astype(jnp.bfloat16)
            y = _rb(jnp.dot(h, w2_ref[...], preferred_element_type=jnp.float32))
            y = _rb(y + b2_ref[...].astype(jnp.float32))
            xs_ref[rows, :] = _rb(x + y)
            return carry
        lax.fori_loop(0, S // TM, body, 0)

    gfnet()
    ffn()
    gfnet()
    ffn()
    o_ref[...] = xs_ref[...].astype(jnp.bfloat16)


@jax.jit
def pallas_interleave_layers__spectral_gfnet__dense_activation_gelu__prompt_kernel(
    A_x, A_w_r, A_w_i, B_x, B_w1, B_b1, B_w2, B_b2):
    fd, gd, m1, m1i, f, fi = _tables()
    x = A_x.reshape(S, D)
    pad = ((0, 0), (0, DP - DF))
    wr = jnp.pad(A_w_r, pad)
    wi = jnp.pad(A_w_i, pad)
    out = pl.pallas_call(
        _kernel,
        out_shape=jax.ShapeDtypeStruct((S, D), jnp.bfloat16),
        scratch_shapes=[
            pltpu.VMEM((S, D), jnp.float32),
            pltpu.VMEM((2, S, DP), jnp.float32),
            pltpu.VMEM((6, S, 128), jnp.float32),
        ],
        compiler_params=pltpu.CompilerParams(vmem_limit_bytes=100 * 1024 * 1024),
    )(x, wr, wi, B_w1, B_b1.reshape(1, F), B_w2, B_b2.reshape(1, D),
      fd, gd, m1, m1i, f, fi)
    return out.reshape(1, S, D)
```

```python
import functools
import numpy as np
import jax
import jax.numpy as jnp
from jax import lax
import jax.experimental.pallas as pl
import jax.experimental.pallas.tpu as pltpu

S, D, F = 2048, 640, 1728
DF = D // 2 + 1
DP = 384
NB, BL = 16, 128
EPS = 1e-5
TM = 256


def _big(m):
    mr, mi = m.real, m.imag
    return np.block([[mr, mi], [-mi, mr]])


@functools.lru_cache(maxsize=None)
def _tables():
    d = np.arange(D)
    l = np.arange(DP)
    ang = 2.0 * np.pi * ((d[:, None] * l[None, :]) % D) / D
    fd = np.zeros((D, 2 * DP))
    fd[:, :DF] = np.cos(ang[:, :DF])
    fd[:, DP + 1:DP + DF - 1] = np.sin(ang[:, 1:DF - 1])
    gd = np.zeros((2 * DP, D))
    c = np.full(DF, 2.0)
    c[0] = c[DF - 1] = 1.0
    gd[:DF, :] = c[:, None] * np.cos(ang.T[:DF]) / (D * S)
    gd[DP + 1:DP + DF - 1, :] = 2.0 * np.sin(ang.T[1:DF - 1]) / (D * S)
    m1 = np.zeros((NB, 2 * BL, 2 * BL))
    m1i = np.zeros((NB, 2 * BL, 2 * BL))
    cc = np.arange(NB)
    for g in range(NB):
        m = np.zeros((BL, BL), np.complex128)
        for a in range(NB):
            for bl in range(8):
                n = BL * a + 8 * g + bl
                m[cc * 8 + bl, a * 8 + bl] = np.exp(-2j * np.pi * ((cc * n) % S) / S)
        m1[g] = _big(m)
        m1i[g] = _big(np.conj(m).T)
    b = np.arange(BL)
    f128 = np.exp(-2j * np.pi * ((b[:, None] * b[None, :]) % BL) / BL)
    bf = jnp.bfloat16
    return (np.asarray(fd, bf), np.asarray(gd, bf), np.asarray(m1, bf),
            np.asarray(m1i, bf), np.asarray(_big(f128), bf),
            np.asarray(_big(np.conj(f128)), bf))


def _ln(x):
    m = jnp.mean(x, axis=-1, keepdims=True)
    xc = x - m
    v = jnp.mean(xc * xc, axis=-1, keepdims=True)
    return xc * lax.rsqrt(v + EPS)


def _rb(x):
    return x.astype(jnp.bfloat16).astype(jnp.float32)


def _kernel(x_ref, wr_ref, wi_ref, w1_ref, b1_ref, w2_ref, b2_ref,
            fd_ref, gd_ref, m1_ref, m1i_ref, f_ref, fi_ref,
            o_ref, xs_ref, u_ref, wf_ref):
    xs_ref[...] = x_ref[...].astype(jnp.float32)
    for k, w_ref in enumerate((wr_ref, wi_ref)):
        for j in range(2):
            wf_ref[3 * k + j] = w_ref[:, j * 128:(j + 1) * 128].astype(jnp.float32)
        wf_ref[3 * k + 2] = jnp.zeros((S, 128), jnp.float32)
        wf_ref[3 * k + 2, :, :DF - 256] = w_ref[:, 256:DF].astype(jnp.float32)

    def gfnet():
        def fwd(g, carry):
            off = pl.multiple_of(g * 8, 8)
            xg = jnp.concatenate(
                [xs_ref[pl.ds(a * BL + off, 8), :] for a in range(NB)], axis=0)
            xn = _ln(xg).astype(jnp.bfloat16)
            pq = jnp.dot(xn, fd_ref[...], preferred_element_type=jnp.float32)
            st = jnp.concatenate([pq[:, :DP], pq[:, DP:]], axis=0).astype(jnp.bfloat16)
            u = jnp.dot(m1_ref[g], st, preferred_element_type=jnp.float32)
            for c in range(NB):
                u_ref[0, pl.ds(c * BL + off, 8), :] = u[c * 8:(c + 1) * 8]
                u_ref[1, pl.ds(c * BL + off, 8), :] = u[BL + c * 8:BL + (c + 1) * 8]
            return carry
        lax.fori_loop(0, NB, fwd, 0)

        def mid(c, carry):
            r0 = pl.multiple_of(c * BL, BL)
            st = jnp.concatenate([u_ref[0, pl.ds(r0, BL), :],
                                  u_ref[1, pl.ds(r0, BL), :]], axis=0).astype(jnp.bfloat16)
            z = jnp.dot(f_ref[...], st, preferred_element_type=jnp.float32)
            p, q = z[:BL], z[BL:]
            wr = jnp.concatenate(
                [wf_ref[j, pl.ds(c, BL, stride=NB), :] for j in range(3)], axis=1)
            wi = jnp.concatenate(
                [wf_ref[3 + j, pl.ds(c, BL, stride=NB), :] for j in range(3)], axis=1)
            p2 = p * wr + q * wi
            q2 = q * wr - p * wi
            st2 = jnp.concatenate([p2, q2], axis=0).astype(jnp.bfloat16)
            v = jnp.dot(fi_ref[...], st2, preferred_element_type=jnp.float32)
            u_ref[0, pl.ds(r0, BL), :] = v[:BL]
            u_ref[1, pl.ds(r0, BL), :] = v[BL:]
            return carry
        lax.fori_loop(0, NB, mid, 0)

        def inv(g, carry):
            off = pl.multiple_of(g * 8, 8)
            st = jnp.concatenate(
                [u_ref[0, pl.ds(c * BL + off, 8), :] for c in range(NB)]
                + [u_ref[1, pl.ds(c * BL + off, 8), :] for c in range(NB)],
                axis=0).astype(jnp.bfloat16)
            t = jnp.dot(m1i_ref[g], st, preferred_element_type=jnp.float32)
            pq = jnp.concatenate([t[:BL], t[BL:]], axis=1).astype(jnp.bfloat16)
            y = _rb(jnp.dot(pq, gd_ref[...], preferred_element_type=jnp.float32))
            for a in range(NB):
                rows = pl.ds(a * BL + off, 8)
                xs_ref[rows, :] = _rb(xs_ref[rows, :] + y[a * 8:(a + 1) * 8])
            return carry
        lax.fori_loop(0, NB, inv, 0)

    def ffn():
        def body(i, carry):
            rows = pl.ds(pl.multiple_of(i * TM, TM), TM)
            x = xs_ref[rows, :]
            xn = _ln(x).astype(jnp.bfloat16)
            h = _rb(jnp.dot(xn, w1_ref[...], preferred_element_type=jnp.float32))
            h = _rb(h + b1_ref[...].astype(jnp.float32))
            h = jax.nn.gelu(h, approximate=True).astype(jnp.bfloat16)
            y = _rb(jnp.dot(h, w2_ref[...], preferred_element_type=jnp.float32))
            y = _rb(y + b2_ref[...].astype(jnp.float32))
            xs_ref[rows, :] = _rb(x + y)
            return carry
        lax.fori_loop(0, S // TM, body, 0)

    gfnet()
    ffn()
    gfnet()
    ffn()
    o_ref[...] = xs_ref[...].astype(jnp.bfloat16)


@jax.jit
def pallas_interleave_layers__spectral_gfnet__dense_activation_gelu__prompt_kernel(
    A_x, A_w_r, A_w_i, B_x, B_w1, B_b1, B_w2, B_b2):
    fd, gd, m1, m1i, f, fi = _tables()
    x = A_x.reshape(S, D)
    wr, wi = A_w_r, A_w_i
    out = pl.pallas_call(
        _kernel,
        out_shape=jax.ShapeDtypeStruct((S, D), jnp.bfloat16),
        scratch_shapes=[
            pltpu.VMEM((S, D), jnp.float32),
            pltpu.VMEM((2, S, DP), jnp.float32),
            pltpu.VMEM((6, S, 128), jnp.float32),
        ],
        compiler_params=pltpu.CompilerParams(vmem_limit_bytes=100 * 1024 * 1024),
    )(x, wr, wi, B_w1, B_b1.reshape(1, F), B_w2, B_b2.reshape(1, D),
      fd, gd, m1, m1i, f, fi)
    return out.reshape(1, S, D)
```

```python
import functools
import numpy as np
import jax
import jax.numpy as jnp
from jax import lax
import jax.experimental.pallas as pl
import jax.experimental.pallas.tpu as pltpu

S, D, F = 2048, 640, 1728
DF = D // 2 + 1
DP = 384
NB, BL = 16, 128
EPS = 1e-5
TM = 512


def _big(m):
    mr, mi = m.real, m.imag
    return np.block([[mr, mi], [-mi, mr]])


@functools.lru_cache(maxsize=None)
def _tables():
    d = np.arange(D)
    l = np.arange(DP)
    ang = 2.0 * np.pi * ((d[:, None] * l[None, :]) % D) / D
    fd = np.zeros((D, 2 * DP))
    fd[:, :DF] = np.cos(ang[:, :DF])
    fd[:, DP + 1:DP + DF - 1] = np.sin(ang[:, 1:DF - 1])
    gd = np.zeros((2 * DP, D))
    c = np.full(DF, 2.0)
    c[0] = c[DF - 1] = 1.0
    gd[:DF, :] = c[:, None] * np.cos(ang.T[:DF]) / (D * S)
    gd[DP + 1:DP + DF - 1, :] = 2.0 * np.sin(ang.T[1:DF - 1]) / (D * S)
    m1 = np.zeros((NB, 2 * BL, 2 * BL))
    m1i = np.zeros((NB, 2 * BL, 2 * BL))
    cc = np.arange(NB)
    for g in range(NB):
        m = np.zeros((BL, BL), np.complex128)
        for a in range(NB):
            for bl in range(8):
                n = BL * a + 8 * g + bl
                m[cc * 8 + bl, a * 8 + bl] = np.exp(-2j * np.pi * ((cc * n) % S) / S)
        m1[g] = _big(m)
        m1i[g] = _big(np.conj(m).T)
    b = np.arange(BL)
    f128 = np.exp(-2j * np.pi * ((b[:, None] * b[None, :]) % BL) / BL)
    bf = jnp.bfloat16
    return (np.asarray(fd, bf), np.asarray(gd, bf), np.asarray(m1, bf),
            np.asarray(m1i, bf), np.asarray(_big(f128), bf),
            np.asarray(_big(np.conj(f128)), bf))


def _ln(x):
    m = jnp.mean(x, axis=-1, keepdims=True)
    xc = x - m
    v = jnp.mean(xc * xc, axis=-1, keepdims=True)
    return xc * lax.rsqrt(v + EPS)


def _rb(x):
    return x.astype(jnp.bfloat16).astype(jnp.float32)


def _kernel(x_ref, wr_ref, wi_ref, w1_ref, b1_ref, w2_ref, b2_ref,
            fd_ref, gd_ref, m1_ref, m1i_ref, f_ref, fi_ref,
            o_ref, xs_ref, u_ref, wf_ref):
    xs_ref[...] = x_ref[...].astype(jnp.float32)
    for k, w_ref in enumerate((wr_ref, wi_ref)):
        for j in range(2):
            wf_ref[3 * k + j] = w_ref[:, j * 128:(j + 1) * 128].astype(jnp.float32)
        wf_ref[3 * k + 2] = jnp.zeros((S, 128), jnp.float32)
        wf_ref[3 * k + 2, :, :DF - 256] = w_ref[:, 256:DF].astype(jnp.float32)

    def gfnet():
        def fwd(g, carry):
            off = pl.multiple_of(g * 8, 8)
            xg = jnp.concatenate(
                [xs_ref[pl.ds(a * BL + off, 8), :] for a in range(NB)], axis=0)
            xn = _ln(xg).astype(jnp.bfloat16)
            pq = jnp.dot(xn, fd_ref[...], preferred_element_type=jnp.float32)
            st = jnp.concatenate([pq[:, :DP], pq[:, DP:]], axis=0).astype(jnp.bfloat16)
            u = jnp.dot(m1_ref[g], st, preferred_element_type=jnp.float32)
            for c in range(NB):
                u_ref[0, pl.ds(c * BL + off, 8), :] = u[c * 8:(c + 1) * 8]
                u_ref[1, pl.ds(c * BL + off, 8), :] = u[BL + c * 8:BL + (c + 1) * 8]
            return carry
        lax.fori_loop(0, NB, fwd, 0, unroll=2)

        def mid(c, carry):
            r0 = pl.multiple_of(c * BL, BL)
            st = jnp.concatenate([u_ref[0, pl.ds(r0, BL), :],
                                  u_ref[1, pl.ds(r0, BL), :]], axis=0).astype(jnp.bfloat16)
            z = jnp.dot(f_ref[...], st, preferred_element_type=jnp.float32)
            p, q = z[:BL], z[BL:]
            wr = jnp.concatenate(
                [wf_ref[j, pl.ds(c, BL, stride=NB), :] for j in range(3)], axis=1)
            wi = jnp.concatenate(
                [wf_ref[3 + j, pl.ds(c, BL, stride=NB), :] for j in range(3)], axis=1)
            p2 = p * wr + q * wi
            q2 = q * wr - p * wi
            st2 = jnp.concatenate([p2, q2], axis=0).astype(jnp.bfloat16)
            v = jnp.dot(fi_ref[...], st2, preferred_element_type=jnp.float32)
            u_ref[0, pl.ds(r0, BL), :] = v[:BL]
            u_ref[1, pl.ds(r0, BL), :] = v[BL:]
            return carry
        lax.fori_loop(0, NB, mid, 0, unroll=2)

        def inv(g, carry):
            off = pl.multiple_of(g * 8, 8)
            st = jnp.concatenate(
                [u_ref[0, pl.ds(c * BL + off, 8), :] for c in range(NB)]
                + [u_ref[1, pl.ds(c * BL + off, 8), :] for c in range(NB)],
                axis=0).astype(jnp.bfloat16)
            t = jnp.dot(m1i_ref[g], st, preferred_element_type=jnp.float32)
            pq = jnp.concatenate([t[:BL], t[BL:]], axis=1).astype(jnp.bfloat16)
            y = _rb(jnp.dot(pq, gd_ref[...], preferred_element_type=jnp.float32))
            for a in range(NB):
                rows = pl.ds(a * BL + off, 8)
                xs_ref[rows, :] = _rb(xs_ref[rows, :] + y[a * 8:(a + 1) * 8])
            return carry
        lax.fori_loop(0, NB, inv, 0, unroll=2)

    def ffn():
        def body(i, carry):
            rows = pl.ds(pl.multiple_of(i * TM, TM), TM)
            x = xs_ref[rows, :]
            xn = _ln(x).astype(jnp.bfloat16)
            h = _rb(jnp.dot(xn, w1_ref[...], preferred_element_type=jnp.float32))
            h = _rb(h + b1_ref[...].astype(jnp.float32))
            h = jax.nn.gelu(h, approximate=True).astype(jnp.bfloat16)
            y = _rb(jnp.dot(h, w2_ref[...], preferred_element_type=jnp.float32))
            y = _rb(y + b2_ref[...].astype(jnp.float32))
            xs_ref[rows, :] = _rb(x + y)
            return carry
        lax.fori_loop(0, S // TM, body, 0)

    gfnet()
    ffn()
    gfnet()
    ffn()
    o_ref[...] = xs_ref[...].astype(jnp.bfloat16)


@jax.jit
def pallas_interleave_layers__spectral_gfnet__dense_activation_gelu__prompt_kernel(
    A_x, A_w_r, A_w_i, B_x, B_w1, B_b1, B_w2, B_b2):
    fd, gd, m1, m1i, f, fi = _tables()
    x = A_x.reshape(S, D)
    wr, wi = A_w_r, A_w_i
    out = pl.pallas_call(
        _kernel,
        out_shape=jax.ShapeDtypeStruct((S, D), jnp.bfloat16),
        scratch_shapes=[
            pltpu.VMEM((S, D), jnp.float32),
            pltpu.VMEM((2, S, DP), jnp.float32),
            pltpu.VMEM((6, S, 128), jnp.float32),
        ],
        compiler_params=pltpu.CompilerParams(vmem_limit_bytes=100 * 1024 * 1024),
    )(x, wr, wi, B_w1, B_b1.reshape(1, F), B_w2, B_b2.reshape(1, D),
      fd, gd, m1, m1i, f, fi)
    return out.reshape(1, S, D)
```
